```python
import jax
import jax.numpy as jnp

def _softmax(x, axis=-1):
    return jax.nn.softmax(x, axis=axis)
def _gelu(x):
    return jax.nn.gelu(x, approximate=True)
def _silu(x):
    return jax.nn.silu(x)
def _sigmoid(x):
    return jax.nn.sigmoid(x)
def _layernorm(x, axis=-1, eps=1e-5):
    m = jnp.mean(x, axis=axis, keepdims=True)
    v = jnp.var(x, axis=axis, keepdims=True)
    return (x - m) / jnp.sqrt(v + eps)
def _scatter_add(tgt, idx, src, axis=0):
    return tgt.at[idx].add(src)
def _segment_sum(src, seg, n):
    return jax.ops.segment_sum(src, seg, n)
class _Rng:
    def __init__(self, key):
        self._k = key
    def _next(self):
        self._k, sub = jax.random.split(self._k)
        return sub
    def normal(self, shape):
        return jax.random.normal(self._next(), shape, dtype=jnp.bfloat16)
    def randint(self, lo, hi, shape):
        return jax.random.randint(self._next(), shape, lo, hi, dtype=jnp.int32)
    def uniform(self, shape, lo=0.0, hi=1.0):
        return jax.random.uniform(self._next(), shape, jnp.bfloat16, lo, hi)
    def permutation(self, n):
        return jax.random.permutation(self._next(), n)


kernel_name = 'interleave_layers__sliding_block__sliding_local_dilated__prompt'

def setup_inputs():
    _rng = _Rng(jax.random.key(int.from_bytes(__import__("os").urandom(4), "little")))
    _w = (lambda a: (lambda t: t.astype(jnp.bfloat16) if jnp.issubdtype(t.dtype, jnp.floating) else t)(jnp.asarray(a)))
    def _A_setup():
        B, S, D = 1, 2048, 1024
        return {
            "x": _w((lambda *s: _rng.normal(s) * 0.05)(B, S, D)),
            "wqkv": _w((lambda *s: _rng.normal(s) * 0.05)(D, 3 * D)),
            "wo": _w((lambda *s: _rng.normal(s) * 0.05)(D, D)),
        }
    _A_in = _A_setup()

    def _B_setup():
        B, S, D = 1, 2048, 1024
        return {
            "x": _w((lambda *s: _rng.normal(s) * 0.05)(B, S, D)),
            "wqkv": _w((lambda *s: _rng.normal(s) * 0.05)(D, 3 * D)),
            "wo": _w((lambda *s: _rng.normal(s) * 0.05)(D, D)),
        }
    _B_in = _B_setup()

    return {
        "A_x": _A_in["x"],
        "A_wqkv": _A_in["wqkv"],
        "A_wo": _A_in["wo"],
        "B_x": _B_in["x"],
        "B_wqkv": _B_in["wqkv"],
        "B_wo": _B_in["wo"],
    }

def reference(A_x, A_wqkv, A_wo, B_x, B_wqkv, B_wo):
    def _A_ref(x, wqkv, wo):
        B, S, D = x.shape
        H = 32; Dh = D // H; W = 256
        qkv = (lambda x, *d: x.transpose(*d))((x @ wqkv).reshape(B, S, 3, H, Dh), 2, 0, 3, 1, 4)
        q, k, v = qkv[0], qkv[1], qkv[2]
        scores = jnp.einsum("bhqd,bhkd->bhqk", q, k) * (Dh ** -0.5)
        idx = jnp.arange(S)
        mask = (idx[:, None] - idx[None, :] >= 0) & (idx[:, None] - idx[None, :] < W)
        scores = jnp.where(mask[None, None], scores, -1e9)
        p = _softmax(scores, axis=-1)
        o = jnp.einsum("bhqk,bhkd->bhqd", p, v)
        return (lambda x, *d: x.transpose(*d))(o, 0, 2, 1, 3).reshape(B, S, D) @ wo

    def _B_ref(x, wqkv, wo):
        B, S, D = x.shape
        H = 32; Dh = D // H
        W, dil = 8, 2
        qkv = (lambda x, *d: x.transpose(*d))((x @ wqkv).reshape(B, S, 3, H, Dh), 2, 0, 3, 1, 4)
        q, k, v = qkv[0], qkv[1], qkv[2]
        scale = Dh ** -0.5
        pos = jnp.arange(S)
        off = jnp.arange(W) * dil
        idx = pos[:, None] - off[None, :]
        mask = idx >= 0
        idx_c = jnp.where(mask, idx, 0).reshape(-1)
        kg = k[:, :, idx_c, :].reshape(B, H, S, W, Dh)
        vg = v[:, :, idx_c, :].reshape(B, H, S, W, Dh)
        logits = jnp.einsum("bhsd,bhswd->bhsw", q, kg) * scale
        logits = jnp.where(mask[None, None, :, :], logits, -1e9)
        attn = _softmax(logits, axis=-1)
        o = jnp.einsum("bhsw,bhswd->bhsd", attn, vg)
        return (lambda x, *d: x.transpose(*d))(o, 0, 2, 1, 3).reshape(B, S, D) @ wo

    x = A_x
    x = x + _A_ref(_layernorm(x, axis=-1), A_wqkv, A_wo)
    x = x + _B_ref(_layernorm(x, axis=-1), B_wqkv, B_wo)
    x = x + _A_ref(_layernorm(x, axis=-1), A_wqkv, A_wo)
    x = x + _B_ref(_layernorm(x, axis=-1), B_wqkv, B_wo)
    return x
```

```python
import functools
import jax
import jax.numpy as jnp
import numpy as np
from jax import lax
import jax.experimental.pallas as pl
import jax.experimental.pallas.tpu as pltpu

S = 2048
D = 1024
BS = 256
NB = S // BS
NG = D // 128
LOG2E = 1.4426950408889634
QSCALE = (32 ** -0.5) * LOG2E
NEG = -1e30
BPAD = 16
RB = 32


def _ln(x):
    m = jnp.mean(x, axis=-1, keepdims=True)
    xc = x - m
    v = jnp.mean(xc * xc, axis=-1, keepdims=True)
    return (xc * lax.rsqrt(v + 1e-5)).astype(jnp.bfloat16)


def _kernel(x_ref, awqkv_hbm, awo_hbm, bwqkv_hbm, bwo_hbm, o_ref,
            xs, awqkv, awo, bwqkv, bwo, ak, av, aq, bq, bk, bv, osc, sems):
    l = pl.program_id(0)
    i = pl.program_id(1)
    row0 = pl.multiple_of(i * BS, BS)

    cps = [pltpu.make_async_copy(awqkv_hbm, awqkv, sems.at[0]),
           pltpu.make_async_copy(awo_hbm, awo, sems.at[1]),
           pltpu.make_async_copy(bwqkv_hbm, bwqkv, sems.at[2]),
           pltpu.make_async_copy(bwo_hbm, bwo, sems.at[3])]

    @pl.when((l == 0) & (i == 0))
    def _():
        for c in cps:
            c.start()
        ak[0:256, :] = jnp.zeros((256, D), jnp.bfloat16)
        av[0:256, :] = jnp.zeros((256, D), jnp.bfloat16)
        bk[:, 0:BPAD, :] = jnp.zeros((NG, BPAD, 128), jnp.float32)
        bv[:, 0:BPAD, :] = jnp.zeros((NG, BPAD, 128), jnp.float32)
        cps[0].wait()
        cps[1].wait()

    @pl.when((l == 1) & (i == 0))
    def _():
        cps[2].wait()
        cps[3].wait()

    @pl.when(l == 0)
    def _():
        xs[pl.ds(row0, BS), :] = x_ref[...].astype(jnp.float32)

    lane = lax.broadcasted_iota(jnp.int32, (128, 128), 1)
    rowi = lax.broadcasted_iota(jnp.int32, (128, 128), 0)

    @pl.when(l % 2 == 0)
    def _layer_a():
        xn = _ln(xs[pl.ds(row0, BS), :])
        q = jnp.dot(xn, awqkv[:, 0:D], preferred_element_type=jnp.float32)
        aq[...] = (q * QSCALE).astype(jnp.bfloat16)
        k = jnp.dot(xn, awqkv[:, D:2 * D], preferred_element_type=jnp.float32)
        ak[pl.ds(row0 + 256, BS), :] = k.astype(jnp.bfloat16)
        v = jnp.dot(xn, awqkv[:, 2 * D:3 * D], preferred_element_type=jnp.float32)
        av[pl.ds(row0 + 256, BS), :] = v.astype(jnp.bfloat16)
        lower = jnp.concatenate([lane <= rowi] * 4, axis=0)
        hm = [(lane // 32) == h for h in range(4)]
        for sb in range(BS // 128):
            q0 = pl.multiple_of(row0 + sb * 128, 128)
            bias0 = jnp.where(q0 >= 256, 0.0, NEG).astype(jnp.float32)
            bias1 = jnp.where(q0 >= 128, 0.0, NEG).astype(jnp.float32)
            for g in range(NG):
                ls = slice(g * 128, (g + 1) * 128)
                qg = aq[sb * 128:(sb + 1) * 128, ls]
                qs = jnp.concatenate([jnp.where(hm[h], qg, jnp.zeros_like(qg)) for h in range(4)], axis=0)
                kw = ak[pl.ds(q0, 384), ls]
                s = lax.dot_general(qs, kw, (((1,), (1,)), ((), ())), preferred_element_type=jnp.float32)
                s0 = s[:, 0:128] + bias0
                s1 = s[:, 128:256] + bias1
                s2 = s[:, 256:384]
                sm = jnp.where(lower, s2, s0)
                m = jnp.max(jnp.maximum(sm, s1), axis=-1, keepdims=True)
                pm = jnp.exp2(sm - m)
                p1 = jnp.exp2(s1 - m)
                den = jnp.sum(pm + p1, axis=-1, keepdims=True)
                pmb = pm.astype(jnp.bfloat16)
                zb = jnp.zeros_like(pmb)
                lowb = lower
                p = jnp.concatenate([jnp.where(lowb, zb, pmb), p1.astype(jnp.bfloat16), jnp.where(lowb, pmb, zb)], axis=1)
                vw = av[pl.ds(q0, 384), ls]
                o = jnp.dot(p, vw, preferred_element_type=jnp.float32)
                o = o * (1.0 / den)
                og = jnp.where(hm[0], o[0:128], jnp.where(hm[1], o[128:256], jnp.where(hm[2], o[256:384], o[384:512])))
                osc[sb * 128:(sb + 1) * 128, ls] = og.astype(jnp.bfloat16)
        xs[pl.ds(row0, BS), :] += jnp.dot(osc[...], awo[...], preferred_element_type=jnp.float32)

    @pl.when(l % 2 == 1)
    def _layer_b():
        xn = _ln(xs[pl.ds(row0, BS), :])
        q = jnp.dot(xn, bwqkv[:, 0:D], preferred_element_type=jnp.float32)
        for g in range(NG):
            bq[g, :, :] = q[:, g * 128:(g + 1) * 128] * QSCALE
        k = jnp.dot(xn, bwqkv[:, D:2 * D], preferred_element_type=jnp.float32)
        for g in range(NG):
            bk[g, pl.ds(row0 + BPAD, BS), :] = k[:, g * 128:(g + 1) * 128]
        v = jnp.dot(xn, bwqkv[:, 2 * D:3 * D], preferred_element_type=jnp.float32)
        for g in range(NG):
            bv[g, pl.ds(row0 + BPAD, BS), :] = v[:, g * 128:(g + 1) * 128]
        bd = ((lane // 32) == (rowi // 32)).astype(jnp.bfloat16)
        rr = lax.broadcasted_iota(jnp.int32, (RB, 128), 0)
        for g in range(NG):
            for c in range(BS // RB):
                r0 = row0 + c * RB
                qc = bq[g, c * RB:(c + 1) * RB, :]
                prods = []
                for w in range(8):
                    kc = bk[g, pl.ds(r0 + BPAD - 2 * w, RB), :]
                    prods.append((qc * kc).astype(jnp.bfloat16))
                lg = jnp.dot(jnp.concatenate(prods, axis=0), bd, preferred_element_type=jnp.float32)
                lgs = []
                for w in range(8):
                    t = lg[w * RB:(w + 1) * RB]
                    if c == 0 and w > 0:
                        t = jnp.where(rr + r0 >= 2 * w, t, NEG)
                    lgs.append(t)
                m = lgs[0]
                for w in range(1, 8):
                    m = jnp.maximum(m, lgs[w])
                den = None
                acc = None
                for w in range(8):
                    e = jnp.exp2(lgs[w] - m)
                    vc = bv[g, pl.ds(r0 + BPAD - 2 * w, RB), :]
                    den = e if den is None else den + e
                    acc = e * vc if acc is None else acc + e * vc
                osc[c * RB:(c + 1) * RB, g * 128:(g + 1) * 128] = (acc * (1.0 / den)).astype(jnp.bfloat16)
        xs[pl.ds(row0, BS), :] += jnp.dot(osc[...], bwo[...], preferred_element_type=jnp.float32)

    @pl.when(l == 3)
    def _():
        o_ref[...] = xs[pl.ds(row0, BS), :].astype(jnp.bfloat16)


@jax.jit
def pallas_interleave_layers__sliding_block__sliding_local_dilated__prompt_kernel(
        A_x, A_wqkv, A_wo, B_x, B_wqkv, B_wo):
    x = A_x.reshape(S, D)
    out = pl.pallas_call(
        _kernel,
        grid=(4, NB),
        in_specs=[pl.BlockSpec((BS, D), lambda l, i: (jnp.where(l == 0, i, NB - 1), 0)),
                  pl.BlockSpec(memory_space=pl.ANY),
                  pl.BlockSpec(memory_space=pl.ANY),
                  pl.BlockSpec(memory_space=pl.ANY),
                  pl.BlockSpec(memory_space=pl.ANY)],
        out_specs=pl.BlockSpec((BS, D), lambda l, i: (jnp.where(l == 3, i, 0), 0)),
        out_shape=jax.ShapeDtypeStruct((S, D), jnp.bfloat16),
        scratch_shapes=[
            pltpu.VMEM((S, D), jnp.float32),
            pltpu.VMEM((D, 3 * D), jnp.bfloat16),
            pltpu.VMEM((D, D), jnp.bfloat16),
            pltpu.VMEM((D, 3 * D), jnp.bfloat16),
            pltpu.VMEM((D, D), jnp.bfloat16),
            pltpu.VMEM((S + 256, D), jnp.bfloat16),
            pltpu.VMEM((S + 256, D), jnp.bfloat16),
            pltpu.VMEM((BS, D), jnp.bfloat16),
            pltpu.VMEM((NG, BS, 128), jnp.float32),
            pltpu.VMEM((NG, S + BPAD, 128), jnp.float32),
            pltpu.VMEM((NG, S + BPAD, 128), jnp.float32),
            pltpu.VMEM((BS, D), jnp.bfloat16),
            pltpu.SemaphoreType.DMA((4,)),
        ],
        compiler_params=pltpu.CompilerParams(
            dimension_semantics=("arbitrary", "arbitrary"),
            vmem_limit_bytes=110 * 1024 * 1024),
    )(x, A_wqkv, A_wo, B_wqkv, B_wo)
    return out.reshape(1, S, D)
```

```python
import functools
import jax
import jax.numpy as jnp
import numpy as np
from jax import lax
import jax.experimental.pallas as pl
import jax.experimental.pallas.tpu as pltpu

S = 2048
D = 1024
BS = 256
NB = S // BS
NG = D // 128
LOG2E = 1.4426950408889634
QSCALE = (32 ** -0.5) * LOG2E
NEG = -1e30
BPAD = 16
RB = 8
NT = 4 * NB
LNG = 1
DEPTH = 2
FOFF = 0
PSPLIT = 1


def _ln(x):
    x = x.astype(jnp.float32)
    m = jnp.mean(x, axis=-1, keepdims=True)
    xc = x - m
    v = jnp.mean(xc * xc, axis=-1, keepdims=True)
    return (xc * lax.rsqrt(v + 1e-5)).astype(jnp.bfloat16)


def _rcp(d):
    r = pl.reciprocal(d, approx=True)
    return r * (2.0 - d * r)


def _kernel(x_hbm, awqkv_hbm, awo_hbm, bwqkv_hbm, bwo_hbm, o_ref,
            xs, wqkv, wo, xn, xn2, osc, sems, *grp):
    aq, ak, av, bq, bk, bv = [grp[j * NG:(j + 1) * NG] for j in range(6)]
    l = pl.program_id(0)
    i = pl.program_id(1)
    t = l * NB + i
    row0 = pl.multiple_of(i * BS, BS)

    def proj(sel, g):
        ys = [jnp.dot(xn[...], wqkv[sel, :, (j * NG + g) * 128:(j * NG + g + 1) * 128],
                      preferred_element_type=jnp.float32) for j in range(3)]
        if sel == 0:
            aq[g][...] = (ys[0] * QSCALE).astype(jnp.bfloat16)
            ak[g][pl.ds(row0 + 256, BS), :] = ys[1].astype(jnp.bfloat16)
            av[g][pl.ds(row0 + 256, BS), :] = ys[2].astype(jnp.bfloat16)
        else:
            bq[g][...] = ys[0] * QSCALE
            bk[g][pl.ds(row0 + BPAD, BS), :] = ys[1]
            bv[g][pl.ds(row0 + BPAD, BS), :] = ys[2]

    def proj_piece(sel, g, j, h):
        n = BS // PSPLIT
        y = jnp.dot(xn[h * n:(h + 1) * n, :], wqkv[sel, :, (j * NG + g) * 128:(j * NG + g + 1) * 128],
                    preferred_element_type=jnp.float32)
        if sel == 1:
            if j == 0:
                bq[g][h * n:(h + 1) * n, :] = y * QSCALE
            elif j == 1:
                bk[g][pl.ds(row0 + BPAD + h * n, n), :] = y
            else:
                bv[g][pl.ds(row0 + BPAD + h * n, n), :] = y

    def ln_for(tt, dst):
        r = pl.multiple_of((tt % NB) * BS, BS)
        dst[...] = _ln(xs[pl.ds(r, BS), :])

    def out_proj(sel):
        y = jnp.dot(osc[...], wo[sel], preferred_element_type=jnp.float32)
        y = (xs[pl.ds(row0, BS), :].astype(jnp.float32) + y).astype(jnp.bfloat16)
        xs[pl.ds(row0, BS), :] = y
        o_ref[...] = y

    cp_x0 = pltpu.make_async_copy(x_hbm.at[pl.ds(0, 2 * BS)], xs.at[pl.ds(0, 2 * BS)], sems.at[0])
    cp_w = pltpu.make_async_copy(awqkv_hbm, wqkv.at[0], sems.at[1])
    cp_x1 = pltpu.make_async_copy(x_hbm.at[pl.ds(2 * BS, S - 2 * BS)], xs.at[pl.ds(2 * BS, S - 2 * BS)], sems.at[4])
    cp_ao = pltpu.make_async_copy(awo_hbm, wo.at[0], sems.at[5])
    cp_bw = pltpu.make_async_copy(bwqkv_hbm, wqkv.at[1], sems.at[6])
    cp_bo = pltpu.make_async_copy(bwo_hbm, wo.at[1], sems.at[7])

    @pl.when(t == 0)
    def _prologue():
        cp_x0.start()
        cp_w.start()
        cp_ao.start()
        for g in range(NG):
            ak[g][0:256, :] = jnp.zeros((256, 128), jnp.bfloat16)
            av[g][0:256, :] = jnp.zeros((256, 128), jnp.bfloat16)
            bk[g][0:BPAD, :] = jnp.zeros((BPAD, 128), jnp.float32)
            bv[g][0:BPAD, :] = jnp.zeros((BPAD, 128), jnp.float32)
        cp_x0.wait()
        ln_for(t, xn)
        cp_w.wait()
        cp_ao.wait()
        cp_x1.start()
        cp_bw.start()
        cp_bo.start()

    @pl.when(t == 1)
    def _():
        cp_x1.wait()

    @pl.when(t == NB)
    def _():
        cp_bw.wait()
        cp_bo.wait()

    lane = lax.broadcasted_iota(jnp.int32, (128, 128), 1)
    rowi = lax.broadcasted_iota(jnp.int32, (128, 128), 0)

    def attn_a(sb, g, consts):
        lower, hmu, hm = consts
        q0 = pl.multiple_of(row0 + sb * 128, 128)
        bias0 = jnp.where(q0 >= 256, 0.0, NEG).astype(jnp.float32)
        bias1 = jnp.where(q0 >= 128, 0.0, NEG).astype(jnp.float32)
        ls = slice(g * 128, (g + 1) * 128)
        qg = pltpu.bitcast(aq[g][sb * 128:(sb + 1) * 128, :], jnp.uint32)
        qs = pltpu.bitcast(jnp.concatenate([qg] * 4, axis=0) & hmu, jnp.bfloat16)
        kw = ak[g][pl.ds(q0, 384), :]
        s = lax.dot_general(qs, kw, (((1,), (1,)), ((), ())), preferred_element_type=jnp.float32)
        s0 = s[:, 0:128] + bias0
        s1 = s[:, 128:256] + bias1
        s2 = s[:, 256:384]
        sm = jnp.where(lower, s2, s0)
        m = jnp.max(jnp.maximum(sm, s1), axis=-1, keepdims=True)
        pm = jnp.exp2(sm - m)
        p1 = jnp.exp2(s1 - m)
        den = jnp.sum(pm + p1, axis=-1, keepdims=True)
        p2 = jnp.where(lower, pm, 0.0)
        p0 = pm - p2
        p = jnp.concatenate([p0, p1, p2], axis=1).astype(jnp.bfloat16)
        vw = av[g][pl.ds(q0, 384), :]
        o = jnp.dot(p, vw, preferred_element_type=jnp.float32)
        og = jnp.where(hm[0], o[0:128], jnp.where(hm[1], o[128:256], jnp.where(hm[2], o[256:384], o[384:512])))
        dg = jnp.where(hm[0], den[0:128], jnp.where(hm[1], den[128:256], jnp.where(hm[2], den[256:384], den[384:512])))
        osc[sb * 128:(sb + 1) * 128, ls] = (og * _rcp(dg)).astype(jnp.bfloat16)

    def attn_b(g, bd, fillers):
        rr = lax.broadcasted_iota(jnp.int32, (RB, 128), 0)
        nch = BS // RB

        def logits(c):
            r0 = row0 + c * RB
            qc = bq[g][c * RB:(c + 1) * RB, :]
            prods = [qc * bk[g][pl.ds(r0 + BPAD - 2 * w, RB), :] for w in range(8)]
            return jnp.dot(jnp.concatenate(prods, axis=0).astype(jnp.bfloat16), bd, preferred_element_type=jnp.float32)

        def finish(c, lg):
            r0 = row0 + c * RB
            lgs = []
            for w in range(8):
                tt = lg[w * RB:(w + 1) * RB]
                if c * RB < 14 and w > 0:
                    tt = jnp.where(rr + r0 >= 2 * w, tt, NEG)
                lgs.append(tt)
            m = lgs[0]
            for w in range(1, 8):
                m = jnp.maximum(m, lgs[w])
            den = None
            acc = None
            for w in range(8):
                e = jnp.exp2(lgs[w] - m)
                vc = bv[g][pl.ds(r0 + BPAD - 2 * w, RB), :]
                den = e if den is None else den + e
                acc = e * vc if acc is None else acc + e * vc
            osc[c * RB:(c + 1) * RB, g * 128:(g + 1) * 128] = (acc * _rcp(den)).astype(jnp.bfloat16)

        fillers = list(fillers)
        every = max(1, nch // max(1, len(fillers)))
        pend = []
        for c in range(nch):
            pend.append((c, logits(c)))
            if c % every == FOFF % every and fillers:
                fillers.pop(0)()
            if len(pend) > DEPTH:
                finish(*pend.pop(0))
        for f in fillers:
            f()
        for p in pend:
            finish(*p)

    @pl.when(l % 2 == 0)
    def _layer_a():
        lower = jnp.concatenate([lane <= rowi] * 4, axis=0)
        lane64 = lax.broadcasted_iota(jnp.int32, (64, 128), 1)
        hmu = jnp.concatenate([jnp.where(lane64 // 32 == h, jnp.uint32(0xFFFFFFFF), jnp.uint32(0)) for h in range(4)], axis=0)
        hm = [(lane // 32) == h for h in range(4)]
        proj(0, 0)
        for g in range(NG):
            if g == LNG:
                ln_for(t + 1, xn2)
            if g + 1 < NG:
                proj(0, g + 1)
            for sb in range(BS // 128):
                attn_a(sb, g, (lower, hmu, hm))
        out_proj(0)
        xn[...] = xn2[...]

    @pl.when(l % 2 == 1)
    def _layer_b():
        bd = ((lane // 32) == (rowi // 32)).astype(jnp.bfloat16)
        proj(1, 0)
        for g in range(NG):
            if g == LNG:
                ln_for(t + 1, xn2)
            fl = []
            if g + 1 < NG:
                fl = [functools.partial(proj_piece, 1, g + 1, j, h) for j in range(3) for h in range(PSPLIT)]
            attn_b(g, bd, fl)
        out_proj(1)
        xn[...] = xn2[...]


@jax.jit
def pallas_interleave_layers__sliding_block__sliding_local_dilated__prompt_kernel(
        A_x, A_wqkv, A_wo, B_x, B_wqkv, B_wo):
    x = A_x.reshape(S, D)
    any_spec = pl.BlockSpec(memory_space=pl.ANY)
    out = pl.pallas_call(
        _kernel,
        grid=(4, NB),
        in_specs=[any_spec] * 5,
        out_specs=pl.BlockSpec((BS, D), lambda l, i: (jnp.where(l == 3, i, 0), 0)),
        out_shape=jax.ShapeDtypeStruct((S, D), jnp.bfloat16),
        scratch_shapes=[
            pltpu.VMEM((S, D), jnp.bfloat16),
            pltpu.VMEM((2, D, 3 * D), jnp.bfloat16),
            pltpu.VMEM((2, D, D), jnp.bfloat16),
            pltpu.VMEM((BS, D), jnp.bfloat16),
            pltpu.VMEM((BS, D), jnp.bfloat16),
            pltpu.VMEM((BS, D), jnp.bfloat16),
            pltpu.SemaphoreType.DMA((8,)),
        ] + [pltpu.VMEM((BS, 128), jnp.bfloat16)] * NG
          + [pltpu.VMEM((S + 256, 128), jnp.bfloat16)] * (2 * NG)
          + [pltpu.VMEM((BS, 128), jnp.float32)] * NG
          + [pltpu.VMEM((S + BPAD, 128), jnp.float32)] * (2 * NG),
        compiler_params=pltpu.CompilerParams(
            dimension_semantics=("arbitrary", "arbitrary"),
            vmem_limit_bytes=110 * 1024 * 1024),
    )(x, A_wqkv, A_wo, B_wqkv, B_wo)
    return out.reshape(1, S, D)
```

```python
import functools
import jax
import jax.numpy as jnp
from jax import lax
import jax.experimental.pallas as pl
import jax.experimental.pallas.tpu as pltpu

S = 2048
D = 1024
BS = 256
NB = S // BS
NG = D // 128
LOG2E = 1.4426950408889634
QSCALE = (32 ** -0.5) * LOG2E
NEG = -1e30
BPAD = 16
RB = 8
NT = 4 * NB
LNC = 16
DEPTH = 2
FOFF = 0
PSPLIT = 1


def _ln(x):
    x = x.astype(jnp.float32)
    m = jnp.mean(x, axis=-1, keepdims=True)
    xc = x - m
    v = jnp.mean(xc * xc, axis=-1, keepdims=True)
    return (xc * lax.rsqrt(v + 1e-5)).astype(jnp.bfloat16)


def _rcp(d):
    r = pl.reciprocal(d, approx=True)
    return r * (2.0 - d * r)


def _kernel(x_hbm, awqkv_hbm, awo_hbm, bwqkv_hbm, bwo_hbm, o_ref,
            xs, wqkv, wo, xn, osc, sems, *grp):
    aq, ak, av, bq, bk, bv = [grp[j * NG:(j + 1) * NG] for j in range(6)]
    l = pl.program_id(0)
    i = pl.program_id(1)
    t = l * NB + i
    row0 = pl.multiple_of(i * BS, BS)

    def proj(sel, g):
        ys = [jnp.dot(xn[...], wqkv[sel, :, (j * NG + g) * 128:(j * NG + g + 1) * 128],
                      preferred_element_type=jnp.float32) for j in range(3)]
        if sel == 0:
            aq[g][...] = (ys[0] * QSCALE).astype(jnp.bfloat16)
            ak[g][pl.ds(row0 + 256, BS), :] = ys[1].astype(jnp.bfloat16)
            av[g][pl.ds(row0 + 256, BS), :] = ys[2].astype(jnp.bfloat16)
        else:
            bq[g][...] = ys[0] * QSCALE
            bk[g][pl.ds(row0 + BPAD, BS), :] = ys[1]
            bv[g][pl.ds(row0 + BPAD, BS), :] = ys[2]

    def proj_piece(sel, g, j, h):
        n = BS // PSPLIT
        y = jnp.dot(xn[h * n:(h + 1) * n, :], wqkv[sel, :, (j * NG + g) * 128:(j * NG + g + 1) * 128],
                    preferred_element_type=jnp.float32)
        if sel == 1:
            if j == 0:
                bq[g][h * n:(h + 1) * n, :] = y * QSCALE
            elif j == 1:
                bk[g][pl.ds(row0 + BPAD + h * n, n), :] = y
            else:
                bv[g][pl.ds(row0 + BPAD + h * n, n), :] = y

    def ln_for(tt, dst):
        r = pl.multiple_of((tt % NB) * BS, BS)
        for c in range(BS // LNC):
            dst[c * LNC:(c + 1) * LNC, :] = _ln(xs[pl.ds(r + c * LNC, LNC), :])

    def out_proj(sel):
        y = jnp.dot(osc[...], wo[sel], preferred_element_type=jnp.float32)
        y = (xs[pl.ds(row0, BS), :].astype(jnp.float32) + y).astype(jnp.bfloat16)
        xs[pl.ds(row0, BS), :] = y
        o_ref[...] = y

    cp_x0 = pltpu.make_async_copy(x_hbm.at[pl.ds(0, 2 * BS)], xs.at[pl.ds(0, 2 * BS)], sems.at[0])
    cp_w = pltpu.make_async_copy(awqkv_hbm, wqkv.at[0], sems.at[1])
    cp_x1 = pltpu.make_async_copy(x_hbm.at[pl.ds(2 * BS, S - 2 * BS)], xs.at[pl.ds(2 * BS, S - 2 * BS)], sems.at[4])
    cp_ao = pltpu.make_async_copy(awo_hbm, wo.at[0], sems.at[5])
    cp_bw = pltpu.make_async_copy(bwqkv_hbm, wqkv.at[1], sems.at[6])
    cp_bo = pltpu.make_async_copy(bwo_hbm, wo.at[1], sems.at[7])

    @pl.when(t == 0)
    def _prologue():
        cp_x0.start()
        cp_w.start()
        cp_ao.start()
        for g in range(NG):
            ak[g][0:256, :] = jnp.zeros((256, 128), jnp.bfloat16)
            av[g][0:256, :] = jnp.zeros((256, 128), jnp.bfloat16)
            bk[g][0:BPAD, :] = jnp.zeros((BPAD, 128), jnp.float32)
            bv[g][0:BPAD, :] = jnp.zeros((BPAD, 128), jnp.float32)
        cp_x0.wait()
        ln_for(t, xn)
        cp_w.wait()
        cp_ao.wait()
        cp_x1.start()
        cp_bw.start()
        cp_bo.start()

    @pl.when(t == 1)
    def _():
        cp_x1.wait()

    @pl.when(t == NB)
    def _():
        cp_bw.wait()
        cp_bo.wait()

    lane = lax.broadcasted_iota(jnp.int32, (128, 128), 1)
    rowi = lax.broadcasted_iota(jnp.int32, (128, 128), 0)

    def attn_a(sb, g, consts):
        lower, hmu, hm = consts
        q0 = pl.multiple_of(row0 + sb * 128, 128)
        bias0 = jnp.where(q0 >= 256, 0.0, NEG).astype(jnp.float32)
        bias1 = jnp.where(q0 >= 128, 0.0, NEG).astype(jnp.float32)
        ls = slice(g * 128, (g + 1) * 128)
        qg = pltpu.bitcast(aq[g][sb * 128:(sb + 1) * 128, :], jnp.uint32)
        qs = pltpu.bitcast(jnp.concatenate([qg] * 4, axis=0) & hmu, jnp.bfloat16)
        kw = ak[g][pl.ds(q0, 384), :]
        s = lax.dot_general(qs, kw, (((1,), (1,)), ((), ())), preferred_element_type=jnp.float32)
        s0 = s[:, 0:128] + bias0
        s1 = s[:, 128:256] + bias1
        s2 = s[:, 256:384]
        sm = jnp.where(lower, s2, s0)
        m = jnp.max(jnp.maximum(sm, s1), axis=-1, keepdims=True)
        pm = jnp.exp2(sm - m)
        p1 = jnp.exp2(s1 - m)
        den = jnp.sum(pm + p1, axis=-1, keepdims=True)
        p2 = jnp.where(lower, pm, 0.0)
        p0 = pm - p2
        p = jnp.concatenate([p0, p1, p2], axis=1).astype(jnp.bfloat16)
        vw = av[g][pl.ds(q0, 384), :]
        o = jnp.dot(p, vw, preferred_element_type=jnp.float32)
        og = jnp.where(hm[0], o[0:128], jnp.where(hm[1], o[128:256], jnp.where(hm[2], o[256:384], o[384:512])))
        dg = jnp.where(hm[0], den[0:128], jnp.where(hm[1], den[128:256], jnp.where(hm[2], den[256:384], den[384:512])))
        osc[sb * 128:(sb + 1) * 128, ls] = (og * _rcp(dg)).astype(jnp.bfloat16)

    def attn_b(g, bd, fillers):
        rr = lax.broadcasted_iota(jnp.int32, (RB, 128), 0)
        nch = BS // RB

        def logits(c):
            r0 = row0 + c * RB
            qc = bq[g][c * RB:(c + 1) * RB, :]
            prods = [qc * bk[g][pl.ds(r0 + BPAD - 2 * w, RB), :] for w in range(8)]
            return jnp.dot(jnp.concatenate(prods, axis=0).astype(jnp.bfloat16), bd, preferred_element_type=jnp.float32)

        def finish(c, lg):
            r0 = row0 + c * RB
            lgs = []
            for w in range(8):
                tt = lg[w * RB:(w + 1) * RB]
                if c * RB < 14 and w > 0:
                    tt = jnp.where(rr + r0 >= 2 * w, tt, NEG)
                lgs.append(tt)
            m = lgs[0]
            for w in range(1, 8):
                m = jnp.maximum(m, lgs[w])
            den = None
            acc = None
            for w in range(8):
                e = jnp.exp2(lgs[w] - m)
                vc = bv[g][pl.ds(r0 + BPAD - 2 * w, RB), :]
                den = e if den is None else den + e
                acc = e * vc if acc is None else acc + e * vc
            osc[c * RB:(c + 1) * RB, g * 128:(g + 1) * 128] = (acc * _rcp(den)).astype(jnp.bfloat16)

        fillers = list(fillers)
        every = max(1, nch // max(1, len(fillers)))
        pend = []
        for c in range(nch):
            pend.append((c, logits(c)))
            if c % every == FOFF % every and fillers:
                fillers.pop(0)()
            if len(pend) > DEPTH:
                finish(*pend.pop(0))
        for f in fillers:
            f()
        for p in pend:
            finish(*p)

    @pl.when(l % 2 == 0)
    def _layer_a():
        lower = jnp.concatenate([lane <= rowi] * 4, axis=0)
        lane64 = lax.broadcasted_iota(jnp.int32, (64, 128), 1)
        hmu = jnp.concatenate([jnp.where(lane64 // 32 == h, jnp.uint32(0xFFFFFFFF), jnp.uint32(0)) for h in range(4)], axis=0)
        hm = [(lane // 32) == h for h in range(4)]
        proj(0, 0)
        for g in range(NG):
            if g + 1 < NG:
                proj(0, g + 1)
            for sb in range(BS // 128):
                attn_a(sb, g, (lower, hmu, hm))
        ln_for(t + 1, xn)
        out_proj(0)

    @pl.when(l % 2 == 1)
    def _layer_b():
        bd = ((lane // 32) == (rowi // 32)).astype(jnp.bfloat16)
        proj(1, 0)
        for g in range(NG):
            fl = []
            if g + 1 < NG:
                fl = [functools.partial(proj_piece, 1, g + 1, j, h) for j in range(3) for h in range(PSPLIT)]
            attn_b(g, bd, fl)
        ln_for(t + 1, xn)
        out_proj(1)


@jax.jit
def pallas_interleave_layers__sliding_block__sliding_local_dilated__prompt_kernel(
        A_x, A_wqkv, A_wo, B_x, B_wqkv, B_wo):
    x = A_x.reshape(S, D)
    any_spec = pl.BlockSpec(memory_space=pl.ANY)
    out = pl.pallas_call(
        _kernel,
        grid=(4, NB),
        in_specs=[any_spec] * 5,
        out_specs=pl.BlockSpec((BS, D), lambda l, i: (jnp.where(l == 3, i, 0), 0)),
        out_shape=jax.ShapeDtypeStruct((S, D), jnp.bfloat16),
        scratch_shapes=[
            pltpu.VMEM((S, D), jnp.bfloat16),
            pltpu.VMEM((2, D, 3 * D), jnp.bfloat16),
            pltpu.VMEM((2, D, D), jnp.bfloat16),
            pltpu.VMEM((BS, D), jnp.bfloat16),
            pltpu.VMEM((BS, D), jnp.bfloat16),
            pltpu.SemaphoreType.DMA((8,)),
        ] + [pltpu.VMEM((BS, 128), jnp.bfloat16)] * NG
          + [pltpu.VMEM((S + 256, 128), jnp.bfloat16)] * (2 * NG)
          + [pltpu.VMEM((BS, 128), jnp.float32)] * NG
          + [pltpu.VMEM((S + BPAD, 128), jnp.float32)] * (2 * NG),
        compiler_params=pltpu.CompilerParams(
            dimension_semantics=("arbitrary", "arbitrary"),
            vmem_limit_bytes=110 * 1024 * 1024),
    )(x, A_wqkv, A_wo, B_wqkv, B_wo)
    return out.reshape(1, S, D)
```
